```python
import os as _os
_os.environ.setdefault("JAX_PLATFORMS", "cpu")
import jax
import jax.numpy as jnp

def _softmax(x, axis=-1):
    return jax.nn.softmax(x, axis=axis)
def _gelu(x):
    return jax.nn.gelu(x, approximate=True)
def _silu(x):
    return jax.nn.silu(x)
def _sigmoid(x):
    return jax.nn.sigmoid(x)
def _layernorm(x, axis=-1, eps=1e-5):
    m = jnp.mean(x, axis=axis, keepdims=True)
    v = jnp.var(x, axis=axis, keepdims=True)
    return (x - m) / jnp.sqrt(v + eps)
def _scatter_add(tgt, idx, src, axis=0):
    return tgt.at[idx].add(src)
def _segment_sum(src, seg, n):
    return jax.ops.segment_sum(src, seg, n)
class _Rng:
    def __init__(self, key):
        self._k = key
    def _next(self):
        self._k, sub = jax.random.split(self._k)
        return sub
    def normal(self, shape):
        return jax.random.normal(self._next(), shape, dtype=jnp.bfloat16)
    def randint(self, lo, hi, shape):
        return jax.random.randint(self._next(), shape, lo, hi, dtype=jnp.int32)
    def uniform(self, shape, lo=0.0, hi=1.0):
        return jax.random.uniform(self._next(), shape, jnp.bfloat16, lo, hi)
    def permutation(self, n):
        return jax.random.permutation(self._next(), n)


kernel_name = 'sequential_preLN__softmax_full_mha__dense_activation_squared_relu__prompt'

def setup_inputs():
    _rng = _Rng(jax.random.key(int.from_bytes(__import__("os").urandom(4), "little")))
    _w = (lambda a: (lambda t: t.astype(jnp.bfloat16) if jnp.issubdtype(t.dtype, jnp.floating) else t)(jnp.asarray(a)))
    def _A_setup():
        B, S, D = 1, 2048, 448
        return {
            "x": _w((lambda *s: _rng.normal(s) * 0.05)(B, S, D)),
            "wqkv": _w((lambda *s: _rng.normal(s) * 0.05)(D, 3 * D)),
            "wo": _w((lambda *s: _rng.normal(s) * 0.05)(D, D)),
        }
    _A_in = _A_setup()

    def _B_setup():
        B, S, D, F = 1, 2048, 448, 1792
        return {
            "x": _w((lambda *s: _rng.normal(s) * 0.05)(B, S, D)),
            "w1": _w((lambda *s: _rng.normal(s) * 0.05)(D, F)),
            "b1": _w((lambda *s: _rng.normal(s) * 0.05)(F)),
            "w2": _w((lambda *s: _rng.normal(s) * 0.05)(F, D)),
            "b2": _w((lambda *s: _rng.normal(s) * 0.05)(D)),
        }
    _B_in = _B_setup()

    return {
        "A_x": _A_in["x"],
        "A_wqkv": _A_in["wqkv"],
        "A_wo": _A_in["wo"],
        "B_x": _B_in["x"],
        "B_w1": _B_in["w1"],
        "B_b1": _B_in["b1"],
        "B_w2": _B_in["w2"],
        "B_b2": _B_in["b2"],
    }

def reference(A_x, A_wqkv, A_wo, B_x, B_w1, B_b1, B_w2, B_b2):
    def _A_ref(x, wqkv, wo):
        B, S, D = x.shape
        H = 16; Dh = D // H
        qkv = (lambda x, *d: x.transpose(*d))((x @ wqkv).reshape(B, S, 3, H, Dh), 2, 0, 3, 1, 4)
        q, k, v = qkv[0], qkv[1], qkv[2]
        scale = Dh ** -0.5
        scores = jnp.einsum("bhqd,bhkd->bhqk", q, k) * scale
        p = _softmax(scores, axis=-1)
        o = jnp.einsum("bhqk,bhkd->bhqd", p, v)
        return (lambda x, *d: x.transpose(*d))(o, 0, 2, 1, 3).reshape(B, S, D) @ wo

    def _B_ref(x, w1, b1, w2, b2):
        h = jnp.einsum("bsd,df->bsf", x, w1) + b1
        zero = jnp.zeros_like(h)
        r = jnp.where(h > zero, h, zero)
        h = r * r
        out = jnp.einsum("bsf,fd->bsd", h, w2) + b2
        return out

    x = A_x
    h = x + _A_ref(_layernorm(x, axis=-1), A_wqkv, A_wo)
    h2 = h + _B_ref(_layernorm(h, axis=-1), B_w1, B_b1, B_w2, B_b2)
    return h2
```

```python
import functools
import math

import jax
import jax.numpy as jnp
from jax import lax
import jax.experimental.pallas as pl
import jax.experimental.pallas.tpu as pltpu

BF = jnp.bfloat16
F32 = jnp.float32
H = 16
EPS = 1e-5


def _dot(a, b):
    return jnp.dot(a, b, preferred_element_type=F32)


def _layernorm_cols(x):
    d = x.shape[0]
    mean = jnp.sum(x, axis=0, keepdims=True) * (1.0 / d)
    xc = x - mean
    var = jnp.sum(xc * xc, axis=0, keepdims=True) * (1.0 / d)
    return xc * lax.rsqrt(var + EPS)


def _kernel(x_hbm, wqkv_hbm, wo_hbm, w1_hbm, b1_ref, w2t_hbm, b2_ref, out_hbm,
            x_s, wqkv_s, wo_s, w1_s, w2t_s,
            wqkvt_s, wot_s, w1t_s, b2_s,
            q_s, k_s, v_s, s_s, m_s, o_s, out_s,
            in_sem, out_sem, *, S, D, F, BQ, CK):
    DH = D // H
    NQ = S // BQ
    G = 4 * DH

    x_cp = [pltpu.make_async_copy(x_hbm.at[:, pl.ds(j * BQ, BQ)], x_s.at[j], in_sem.at[j])
            for j in range(NQ)]
    wqkv_cp = pltpu.make_async_copy(wqkv_hbm, wqkv_s, in_sem.at[NQ])
    wo_cp = pltpu.make_async_copy(wo_hbm, wo_s, in_sem.at[NQ + 1])
    w1_cp = pltpu.make_async_copy(w1_hbm, w1_s, in_sem.at[NQ + 2])
    w2_cp = pltpu.make_async_copy(w2t_hbm, w2t_s, in_sem.at[NQ + 3])
    wqkv_cp.start()
    for c in x_cp:
        c.start()
    wo_cp.start()
    w1_cp.start()
    w2_cp.start()

    wqkv_cp.wait()
    wqkvt_s[...] = wqkv_s[...].T
    qscale = (DH ** -0.5) * math.log2(math.e)
    row32 = lax.broadcasted_iota(jnp.int32, (32, BQ), 0)
    for j in range(NQ):
        x_cp[j].wait()
        y = _layernorm_cols(x_s[j].astype(F32)).astype(BF)
        qkv = _dot(wqkvt_s[...], y)
        cols = pl.ds(j * BQ, BQ)
        for g in range(4):
            q_s[g, j] = (qkv[g * G:g * G + 128] * qscale).astype(BF)
            k_s[g, cols, :] = qkv[D + g * G:D + g * G + 128].T.astype(BF)
        for h in range(H):
            lo = (h * DH) // 8 * 8
            off = h * DH - lo
            win = qkv[2 * D + lo:2 * D + lo + 32]
            keep = (row32 >= off) & (row32 < off + DH)
            v_s[h, :, cols] = jnp.where(keep, win, 1.0).astype(BF)

    row128 = lax.broadcasted_iota(jnp.int32, (128, BQ), 0)

    def step(ha, hb, j):
        if ha is not None:
            g = ha // 4
            lo = (ha % 4) * DH
            qw = jnp.where((row128 >= lo) & (row128 < lo + DH), q_s[g, j].astype(F32), 0.0).astype(BF)
        if hb is not None:
            mb = m_s[j]
        m = acc = None
        for c in range(S // CK):
            ks = pl.ds(c * CK, CK)
            if hb is not None:
                p = jnp.exp2(s_s[j, ks, :] - mb).astype(BF)
            if ha is not None:
                s = _dot(k_s[g, ks, :], qw)
                s_s[j, ks, :] = s
                mc = jnp.max(s.reshape(CK // 8, 8, BQ), axis=0)
                m = mc if m is None else jnp.maximum(m, mc)
            if hb is not None:
                d = _dot(v_s[hb, :, ks], p)
                acc = d if acc is None else acc + d
        if hb is not None:
            o_s[hb, j] = acc
        if ha is not None:
            m_s[j] = jnp.max(m, axis=0, keepdims=True)

    for j in range(NQ):
        step(0, None, j)

    wo_cp.wait()
    w1_cp.wait()
    w2_cp.wait()
    wot_s[...] = wo_s[...].T
    b1 = b1_ref[...].astype(F32).reshape(1, F)
    row16 = lax.broadcasted_iota(jnp.int32, (16, F), 0)
    b1_rows = jnp.where(row16 == 0, b1, 0.0).astype(BF)
    w1t_s[...] = jnp.concatenate([w1_s[...], b1_rows], axis=0).T
    b2 = b2_ref[...].astype(F32).reshape(1, D)
    b2_s[...] = jnp.broadcast_to(b2, (128, D)).T

    def body(h, carry):
        for j in range(NQ):
            step(h + 1, h, j)
        return carry

    lax.fori_loop(0, H - 1, body, 0)

    row8 = lax.broadcasted_iota(jnp.int32, (8, BQ), 0)

    def attn_out(j):
        parts = []
        for h in range(0, H, 2):
            e = o_s[h, j]
            o = o_s[h + 1, j]
            e = e * (1.0 / e[31:32])
            o = o * (1.0 / o[0:1])
            parts += [e[:24], jnp.where(row8 < 4, e[24:], o[:8]), o[8:]]
        a = jnp.concatenate(parts, axis=0).astype(BF)
        return x_s[j].astype(F32) + _dot(wot_s[...], a)

    def ffn(j, hres):
        y = _layernorm_cols(hres).astype(BF)
        y = jnp.concatenate([y, jnp.ones((16, BQ), BF)], axis=0)
        u = jnp.maximum(_dot(w1t_s[...], y), 0.0)
        u = (u * u).astype(BF)
        res = hres + jnp.tile(b2_s[...], (1, BQ // 128)) + _dot(w2t_s[...], u)
        out_s[j] = res.astype(BF)
        cp = pltpu.make_async_copy(out_s.at[j], out_hbm.at[:, pl.ds(j * BQ, BQ)], out_sem.at[j])
        cp.start()
        return cp

    step(None, H - 1, 0)
    hres = attn_out(0)
    cps = []
    for j in range(NQ):
        nxt = None
        if j + 1 < NQ:
            step(None, H - 1, j + 1)
            nxt = attn_out(j + 1)
        cps.append(ffn(j, hres))
        hres = nxt
    for cp in cps:
        cp.wait()


@jax.jit
def pallas_sequential_preLN__softmax_full_mha__dense_activation_squared_relu__prompt_kernel(
        A_x, A_wqkv, A_wo, B_x, B_w1, B_b1, B_w2, B_b2):
    BQ, CK = 512, 128
    del B_x
    _, S, D = A_x.shape
    F = B_w1.shape[1]
    NQ = S // BQ
    hbm = pl.BlockSpec(memory_space=pltpu.HBM)
    vmem = pl.BlockSpec(memory_space=pltpu.VMEM)
    out_t = pl.pallas_call(
        functools.partial(_kernel, S=S, D=D, F=F, BQ=BQ, CK=CK),
        out_shape=jax.ShapeDtypeStruct((D, S), A_x.dtype),
        in_specs=[hbm, hbm, hbm, hbm, vmem, hbm, vmem],
        out_specs=hbm,
        scratch_shapes=[
            pltpu.VMEM((NQ, D, BQ), BF),
            pltpu.VMEM((D, 3 * D), BF),
            pltpu.VMEM((D, D), BF),
            pltpu.VMEM((D, F), BF),
            pltpu.VMEM((D, F), BF),
            pltpu.VMEM((3 * D, D), BF),
            pltpu.VMEM((D, D), BF),
            pltpu.VMEM((F, D + 16), BF),
            pltpu.VMEM((D, 128), F32),
            pltpu.VMEM((4, NQ, 128, BQ), BF),
            pltpu.VMEM((4, S, 128), BF),
            pltpu.VMEM((H, 32, S), BF),
            pltpu.VMEM((NQ, S, BQ), F32),
            pltpu.VMEM((NQ, 1, BQ), F32),
            pltpu.VMEM((H, NQ, 32, BQ), F32),
            pltpu.VMEM((NQ, D, BQ), BF),
            pltpu.SemaphoreType.DMA((NQ + 4,)),
            pltpu.SemaphoreType.DMA((NQ,)),
        ],
        compiler_params=pltpu.CompilerParams(vmem_limit_bytes=100 << 20),
    )(A_x[0].T, A_wqkv, A_wo, B_w1, B_b1, B_w2.T, B_b2)
    return out_t.T[None]
```

```python
import functools
import math

import jax
import jax.numpy as jnp
from jax import lax
import jax.experimental.pallas as pl
import jax.experimental.pallas.tpu as pltpu

BF = jnp.bfloat16
F32 = jnp.float32
U32 = jnp.uint32
H = 16
EPS = 1e-5
K1 = 256


def _dot(a, b):
    return jnp.dot(a, b, preferred_element_type=F32)


def _pack(x):
    return pltpu.bitcast(x.astype(BF), U32)


def _unpack(x):
    return pltpu.bitcast(x, BF)


def _put(ref, r0, c0, val, after=None):
    rows, cols = val.shape
    mask = lax.broadcasted_iota(jnp.int32, (rows, 128), 1) >= 0
    if after is not None:
        bits = lax.bitcast_convert_type(after, jnp.int32) | 1
        mask = jnp.tile(bits, (rows // 8, 1)) != 0
    for c in range(0, cols, 128):
        pltpu.store(ref.at[pl.ds(r0, rows), pl.ds(c0 + c, 128)], val[:, c:c + 128], mask=mask)


def _pad_to(x, n, axis):
    if x.shape[axis] == n:
        return x
    shape = list(x.shape)
    shape[axis] = n - x.shape[axis]
    return jnp.concatenate([x, jnp.zeros(shape, x.dtype)], axis=axis)


def _fold(v):
    return jnp.sum(v.reshape(v.shape[0] // 8, 8, v.shape[1]), axis=0)


def _strassen_lhs(halves, rows, k1, dst, m, r0):
    halves = functools.cache(halves)

    def job(r, c, after):
        top, bot = halves()

        def blk(a, c0):
            return _pad_to(a[r:r + 16, c0 + c:min(c0 + c + 128, a.shape[1])].astype(F32), 128, 1)
        a11, a12, a21, a22 = blk(top, 0), blk(top, k1), blk(bot, 0), blk(bot, k1)
        for i, v in enumerate((a11 + a22, a21 + a22, a11, a22, a11 + a12, a21 - a11, a12 - a22)):
            _put(dst, (i * m + r0 + r) // 2, c, _pack(v), after)
    return [functools.partial(job, r, c) for c in range(0, k1, 128) for r in range(0, rows, 16)]


def _strassen_rhs(get, k1, k2, n, dst, r0=0, rows=None):
    def job(r, c, after):
        b11, b12 = get(0, 0, r, c), get(0, 1, r, c)
        if r < k2:
            b21, b22 = get(1, 0, r, c), get(1, 1, r, c)
            ops = (b11 + b22, b11, b12 - b22, b21 - b11, b22, b11 + b12, b21 + b22)
        else:
            ops = (b11, b11, b12, None, None, b11 + b12, None)
        for i, v in enumerate(ops):
            if v is not None:
                _put(dst, (i * k1 + r) // 2, c, _pack(v), after)
    return [functools.partial(job, r, c)
            for r in range(r0, k1 if rows is None else r0 + rows, 16) for c in range(0, n, 128)]


def _strassen(a_ref, b_ref, t_ref, m, r0, rows, k1, k2, emit, mid=None):
    n = b_ref.shape[1]

    def prod(i):
        k = k2 if i in (3, 4, 6) else k1
        b = _pad_to(b_ref[pl.ds(i * k1 // 2, k // 2), :], k1 // 2, 0)
        return _dot(_unpack(a_ref[pl.ds((i * m + r0) // 2, rows // 2), :]), _unpack(b))

    def put(i, v):
        _put(t_ref, 0, i * n, v)

    def get(i):
        return t_ref[pl.ds(0, rows), pl.ds(i * n, n)]

    p = prod(6)
    if mid is not None:
        mid()
    put(0, p)
    yield p
    p = prod(4)
    put(0, get(0) - p)
    put(1, p)
    yield p
    p = prod(2)
    emit(0, 1, get(1) + p)
    put(1, p)
    yield p
    p = prod(3)
    put(0, get(0) + p)
    put(2, p)
    yield p
    p = prod(1)
    emit(1, 0, get(2) + p)
    put(1, get(1) - p)
    yield p
    p = prod(0)
    emit(0, 0, get(0) + p)
    put(1, get(1) + p)
    yield p
    p = prod(5)
    emit(1, 1, get(1) + p)
    yield p


def _run(gen, jobs=(), slots=1, extra=None, per=0):
    jobs = list(jobs)
    done = 0
    for i, p in enumerate(gen):
        upto = len(jobs) * min(i + 1, slots) // slots
        for k in range(done, upto):
            r = (k - done) * (p.shape[0] // 8) // (upto - done) * 8
            jobs[k](p[r:r + 8, :128])
        done = upto
        for _ in range(per):
            next(extra, None)
    assert done == len(jobs)


def _now(jobs):
    for job in jobs:
        job(None)


def _chain(*gens):
    for g in gens:
        yield from g


def _kernel(x_hbm, wqkv_hbm, wo_hbm, w1_hbm, b1_hbm, w2t_hbm, b2_hbm, out_hbm,
            x_s, wqkv_s, wo_s, w1_s, w2t_s, b1_s, b2_s,
            aqkv_s, ao_s, a1_s, a2_s, b2c_s,
            y_s, u_s, ur_s, t_s, c_s, h_s, qkv_s,
            q_s, k_s, v_s, s_s, m_s, o_s, out_s,
            in_sem, out_sem, *, S, D, F, BQ, CK):
    DH = D // H
    NQ = S // BQ
    G = 4 * DH
    HB = BQ // 2
    WCH = [(0, 256), (256, 256), (512, 256), (768, 256), (1024, 3 * D - 1024)]

    copies = []

    def copy_in(src, dst):
        copies.append(pltpu.make_async_copy(src, dst, in_sem.at[len(copies)]))
        return copies[-1]

    x_cp = [copy_in(x_hbm.at[:, pl.ds(j * BQ, BQ)], x_s.at[:, pl.ds(j * BQ, BQ)]) for j in range(1, NQ)]
    x0_cp = [copy_in(x_hbm.at[:, pl.ds(c, HB)], x_s.at[:, pl.ds(c, HB)]) for c in (0, HB)]
    w_cp = [copy_in(wqkv_hbm.at[:, pl.ds(c, n)], wqkv_s.at[:, pl.ds(c, n)]) for c, n in WCH]
    late_cp = [copy_in(wo_hbm, wo_s), copy_in(w1_hbm, w1_s), copy_in(w2t_hbm, w2t_s),
               copy_in(b1_hbm, b1_s), copy_in(b2_hbm, b2_s)]

    def accumulate(table, key, v):
        table[key] = table[key] + v if key in table else v

    def centre_jobs(j, tiles, totals, squares):
        @functools.cache
        def mean(c):
            return jnp.sum(totals[j, c], axis=0, keepdims=True) * (1.0 / D)

        def job(r, c, after):
            xc = h_s[pl.ds(r, 32), pl.ds(j * BQ + c, 128)] - mean(c)
            _put(c_s, r, c, xc, after)
            accumulate(squares, c, _fold(xc * xc))
        return [functools.partial(job, r, c) for c in tiles for r in range(0, D, 32)]

    def normed_jobs(squares, dst, bias_row):
        @functools.cache
        def rstd(c):
            return lax.rsqrt(jnp.sum(squares[c], axis=0, keepdims=True) * (1.0 / D) + EPS)

        def get(bi, bj, r, c):
            r, c = bi * K1 + r, bj * HB + c
            if r >= D:
                return jnp.ones((16, 128), F32)
            return c_s[pl.ds(r, 16), pl.ds(c, 128)] * rstd(c)
        return _strassen_rhs(get, K1, D - K1 + (16 if bias_row else 0), HB, dst)

    qscale = (DH ** -0.5) * math.log2(math.e)
    row32 = lax.broadcasted_iota(jnp.int32, (32, BQ), 0)
    all_tiles = range(0, BQ, 128)

    def widen_jobs(j, tiles, totals):
        def job(r, c, after):
            x = x_s[pl.ds(r, 32), pl.ds(j * BQ + c, 128)].astype(F32)
            _put(h_s, r, j * BQ + c, x, after)
            accumulate(totals, (j, c), _fold(x))
        return [functools.partial(job, r, c) for c in tiles for r in range(0, D, 32)]

    def ln1(j):
        totals, squares = {}, {}
        return (widen_jobs(j, all_tiles, totals) + centre_jobs(j, all_tiles, totals, squares)
                + normed_jobs(squares, y_s.at[j % 2], False))

    def qkv_chunk(j, i, mid=None):
        c0, n = WCH[i]

        def emit(bi, bj, v):
            _put(qkv_s, c0 + bi * (n // 2), bj * HB, v)
        return _strassen(aqkv_s, y_s.at[j % 2], t_s, 3 * D // 2, c0 // 2, n // 2, K1, D - K1, emit, mid)

    def qkv_finish(j):
        cols = pl.ds(j * BQ, BQ)
        for g in range(4):
            _put(q_s, g * 64, j * BQ, _pack(qkv_s[pl.ds(g * G, 128), :] * qscale))
            _put(k_s, (g * S + j * BQ) // 2, 0, _pack(qkv_s[pl.ds(D + g * G, 128), :].astype(BF).T))
        for h in range(H):
            lo = (h * DH) // 8 * 8
            off = h * DH - lo
            keep = (row32 >= off) & (row32 < off + DH)
            v_s[pl.ds(h * 16, 16), cols] = _pack(jnp.where(keep, qkv_s[pl.ds(2 * D + lo, 32), :], 1.0))

    def wqkv_prep(i):
        c0, n = WCH[i]

        def halves():
            wt = wqkv_s[:, pl.ds(c0, n)].T
            return wt[:n // 2], wt[n // 2:]
        return _strassen_lhs(halves, n // 2, K1, aqkv_s, 3 * D // 2, c0 // 2)

    def then(wait, start):
        def fn():
            for c in wait:
                c.wait()
            for c in start:
                c.start()
        return fn

    x0_cp[0].start()
    x0_cp[1].start()
    w_cp[0].start()
    then(x0_cp[:1], w_cp[1:2])()
    totals, squares = {}, {}
    tiles = range(0, HB, 128)
    _now(widen_jobs(0, tiles, totals) + centre_jobs(0, tiles, totals, squares))
    then([x0_cp[1], w_cp[0]], w_cp[2:3])()
    tiles = range(HB, BQ, 128)
    _now(widen_jobs(0, tiles, totals) + centre_jobs(0, tiles, totals, squares))
    _now(normed_jobs(squares, y_s.at[0], False) + wqkv_prep(0))
    _run(qkv_chunk(0, 0, then(w_cp[1:2], w_cp[3:])))
    _now(wqkv_prep(1))
    _run(qkv_chunk(0, 1, then(w_cp[2:3], x_cp[:1])))
    _now(wqkv_prep(2))
    _run(qkv_chunk(0, 2, then(w_cp[3:], x_cp[1:])))
    _now(wqkv_prep(3) + wqkv_prep(4))
    _run(_chain(qkv_chunk(0, 3, then(x_cp[:1], [])), qkv_chunk(0, 4)), ln1(1), 13)
    qkv_finish(0)
    for j in range(1, NQ):
        _run(qkv_chunk(j, 0))
        _run(_chain(*[qkv_chunk(j, i, then(x_cp[1:], late_cp) if (j, i) == (1, 1) else None) for i in range(1, 5)]),
             ln1(j + 1) if j + 1 < NQ else (), 26)
        qkv_finish(j)

    row64 = lax.broadcasted_iota(jnp.int32, (64, BQ), 0)
    row8 = lax.broadcasted_iota(jnp.int32, (8, 128), 0)

    def aligned(i, n):
        return i if isinstance(i, int) else pl.multiple_of(i, n)

    def step(ha, hb, j):
        cols = pl.ds(j * BQ, BQ)
        if ha is not None:
            g = ha // 4
            lo = (ha % 4) * (DH // 2)
            qw = _unpack(jnp.where((row64 >= lo) & (row64 < lo + DH // 2),
                                   q_s[pl.ds(aligned(g * 64, 64), 64), cols], jnp.zeros((), U32)))
        if hb is not None:
            mb = m_s[j]
        m = acc = None
        for c in range(S // CK):
            ks = pl.ds(c * CK, CK)
            if hb is not None:
                p = jnp.exp2(s_s[j, ks, :] - mb).astype(BF)
            if ha is not None:
                s = _dot(_unpack(k_s[pl.ds(aligned(g * (S // 2) + c * CK // 2, CK // 2), CK // 2), :]), qw)
                s_s[j, ks, :] = s
                mc = jnp.max(s.reshape(CK // 8, 8, BQ), axis=0)
                m = mc if m is None else jnp.maximum(m, mc)
            if hb is not None:
                d = _dot(_unpack(v_s[pl.ds(aligned(hb * 16, 16), 16), ks]), p)
                acc = d if acc is None else acc + d
            yield d if ha is None else s
        if hb is not None:
            _put(o_s, aligned(hb * 32, 32), j * BQ, acc)
        if ha is not None:
            m_s[j] = jnp.max(m, axis=0, keepdims=True)

    def prep_wo():
        b2 = b2_s[...].astype(F32).reshape(1, D)
        b2c_s[...] = jnp.broadcast_to(b2, (128, D)).T

        def halves():
            wt = wo_s[...].T
            return wt[:D // 2], wt[D // 2:]
        return _strassen_lhs(halves, D // 2, K1, ao_s, D // 2, 0)

    def prep_w1(c):
        b1 = b1_s[...].astype(F32).reshape(1, F)
        row16 = lax.broadcasted_iota(jnp.int32, (16, 128), 0)

        def cols_t(c):
            b1_rows = jnp.where(row16 == 0, b1[:, c:c + 128], 0.0).astype(BF)
            return jnp.concatenate([w1_s[:, pl.ds(c, 128)], b1_rows], axis=0).T
        return _strassen_lhs(lambda: (cols_t(c), cols_t(F // 2 + c)), 128, K1, a1_s, F // 2, c)

    def prep_w2():
        return _strassen_lhs(lambda: (w2t_s.at[pl.ds(0, D // 2)], w2t_s.at[pl.ds(D // 2, D // 2)]),
                             D // 2, F // 2, a2_s, D // 2, 0)

    for c in late_cp:
        c.wait()
    jobs = prep_w2() + prep_wo() + [job for c in range(0, F // 2, 128) for job in prep_w1(c)]
    _run(_chain(*[step(0, None, j) for j in range(NQ)]), jobs, NQ * S // CK - 1)

    def body(h, carry):
        for j in range(NQ):
            _run(step(h + 1, h, j))
        return carry

    lax.fori_loop(0, H - 1, body, 0)

    totals = {}

    def heads_jobs(j):
        @functools.cache
        def inv(h, c):
            den = o_s[pl.ds(h * 32 + (0 if h % 2 else 31), 1), pl.ds(j * BQ + c, 128)]
            r = pl.reciprocal(den, approx=True)
            return r * (2.0 - den * r)

        def part(h, r, c):
            return o_s[pl.ds(h * 32 + r - (h * DH) // 8 * 8, 8), pl.ds(j * BQ + c, 128)] * inv(h, c)

        def rows8(r, c):
            h0, h1 = r // DH, (r + 7) // DH
            if h0 == h1:
                return part(h0, r, c)
            return jnp.where(row8 < h1 * DH - r, part(h0, r, c), part(h1, r, c))

        def get(bi, bj, r, c):
            r, c = bi * K1 + r, bj * HB + c
            return jnp.concatenate([rows8(r, c), rows8(r + 8, c)], axis=0)
        return _strassen_rhs(get, K1, D - K1, HB, y_s.at[2 + j % 2])

    def attn_out(j):
        def emit(bi, bj, v):
            r, c = bi * (D // 2), j * BQ + bj * HB
            v = v + h_s[pl.ds(r, D // 2), pl.ds(c, HB)]
            _put(h_s, r, c, v)
            for t in range(0, HB, 128):
                accumulate(totals, (j, bj * HB + t), _fold(v[:, t:t + 128]))
        return _strassen(ao_s, y_s.at[2 + j % 2], t_s, D // 2, 0, D // 2, K1, D - K1, emit)

    def ln2(j):
        squares = {}
        return centre_jobs(j, all_tiles, totals, squares) + normed_jobs(squares, y_s.at[j % 2], True)

    def up(j):
        last = {}

        def emit(bi, bj, v):
            v = jnp.maximum(v, 0.0)
            v = v * v
            if (bi, bj) == (1, 1):
                last[0] = v
            else:
                _put(u_s, 0, (2 * bi + bj) * HB, v)
        yield from _strassen(a1_s, y_s.at[j % 2], t_s, F // 2, 0, F // 2, K1, D - K1 + 16, emit)

        def get(bi, bj, r, c):
            if (bi, bj) == (1, 1):
                return last[0][r:r + 16, c:c + 128]
            return u_s[pl.ds(r, 16), pl.ds((2 * bi + bj) * HB + c, 128)]
        _now(_strassen_rhs(get, F // 2, F // 2, HB, ur_s.at[j % 2]))

    out_cp = []

    def down(j):
        def emit(bi, bj, v):
            rows, cols = pl.ds(bi * (D // 2), D // 2), pl.ds(j * BQ + bj * HB, HB)
            out_s[rows, cols] = (v + h_s[rows, cols] + jnp.tile(b2c_s[rows, :], (1, HB // 128))).astype(BF)
            if j == NQ - 1:
                out_cp.append(pltpu.make_async_copy(out_s.at[rows, cols], out_hbm.at[rows, cols],
                                                    out_sem.at[len(out_cp)]))
                out_cp[-1].start()
        yield from _strassen(a2_s, ur_s.at[j % 2], t_s, D // 2, 0, D // 2, F // 2, F // 2, emit)
        if j < NQ - 1:
            cols = pl.ds(j * BQ, BQ)
            out_cp.append(pltpu.make_async_copy(out_s.at[:, cols], out_hbm.at[:, cols], out_sem.at[len(out_cp)]))
            out_cp[-1].start()

    _run(step(None, H - 1, 0))
    _run(step(None, H - 1, 1), heads_jobs(0), 12)
    gen = step(None, H - 1, 2)
    _run(attn_out(0), heads_jobs(1), 5, gen, 1)
    _run(attn_out(1), ln2(0), 6, gen, 1)
    _run(up(0), ln2(1), 6, gen, 1)
    _run(gen)
    gen = step(None, H - 1, 3)
    _run(up(1), heads_jobs(2), 6, gen, 1)
    _run(attn_out(2), (), 1, gen, 1)
    _run(down(0), ln2(2), 6, gen, 1)
    _run(gen)
    _run(up(2), heads_jobs(3), 6)
    _run(attn_out(3))
    _run(down(1), ln2(3), 6)
    _run(up(3))
    _run(down(2))
    _run(down(3))
    for cp in out_cp:
        cp.wait()


@jax.jit
def pallas_sequential_preLN__softmax_full_mha__dense_activation_squared_relu__prompt_kernel(
        A_x, A_wqkv, A_wo, B_x, B_w1, B_b1, B_w2, B_b2):
    BQ = 512
    CK = 128
    flags = None
    del B_x
    _, S, D = A_x.shape
    F = B_w1.shape[1]
    NQ = S // BQ
    hbm = pl.BlockSpec(memory_space=pltpu.HBM)
    out_t = pl.pallas_call(
        functools.partial(_kernel, S=S, D=D, F=F, BQ=BQ, CK=CK),
        out_shape=jax.ShapeDtypeStruct((D, S), A_x.dtype),
        in_specs=[hbm] * 7,
        out_specs=hbm,
        scratch_shapes=[
            pltpu.VMEM((D, S), BF),
            pltpu.VMEM((D, 3 * D), BF),
            pltpu.VMEM((D, D), BF),
            pltpu.VMEM((D, F), BF),
            pltpu.VMEM((D, F), BF),
            pltpu.VMEM((F,), BF),
            pltpu.VMEM((D,), BF),
            pltpu.VMEM((7 * 3 * D // 4, K1), U32),
            pltpu.VMEM((7 * D // 4, K1), U32),
            pltpu.VMEM((7 * F // 4, K1), U32),
            pltpu.VMEM((7 * D // 4, F // 2), U32),
            pltpu.VMEM((D, 128), F32),
            pltpu.VMEM((4, 7 * K1 // 2, BQ // 2), U32),
            pltpu.VMEM((F // 2, 3 * BQ // 2), F32),
            pltpu.VMEM((2, 7 * F // 4, BQ // 2), U32),
            pltpu.VMEM((F // 2, 3 * BQ // 2), F32),
            pltpu.VMEM((D, BQ), F32),
            pltpu.VMEM((D, S), F32),
            pltpu.VMEM((3 * D, BQ), F32),
            pltpu.VMEM((4 * 64, S), U32),
            pltpu.VMEM((4 * S // 2, 128), U32),
            pltpu.VMEM((H * 16, S), U32),
            pltpu.VMEM((NQ, S, BQ), F32),
            pltpu.VMEM((NQ, 1, BQ), F32),
            pltpu.VMEM((H * 32, S), F32),
            pltpu.VMEM((D, S), BF),
            pltpu.SemaphoreType.DMA((NQ + 11,)),
            pltpu.SemaphoreType.DMA((NQ + 3,)),
        ],
        compiler_params=pltpu.CompilerParams(vmem_limit_bytes=100 << 20, flags=flags),
    )(A_x[0].T, A_wqkv, A_wo, B_w1, B_b1, B_w2.T, B_b2)
    return out_t.T[None]
```

```python
import functools
import math

import jax
import jax.numpy as jnp
from jax import lax
import jax.experimental.pallas as pl
import jax.experimental.pallas.tpu as pltpu

BF = jnp.bfloat16
F32 = jnp.float32
U32 = jnp.uint32
H = 16
EPS = 1e-5
BQ = 512
HB = BQ // 2
K1 = 256
SAFE = 2.0 ** 60

_LHS = (((1, 0, 0), (1, 1, 1)), ((1, 1, 0), (1, 1, 1)), ((1, 0, 0),), ((1, 1, 1),),
        ((1, 0, 0), (1, 0, 1)), ((1, 1, 0), (-1, 0, 0)), ((1, 0, 1), (-1, 1, 1)))
_RHS = (((1, 0, 0), (1, 1, 1)), ((1, 0, 0),), ((1, 0, 1), (-1, 1, 1)), ((1, 1, 0), (-1, 0, 0)),
        ((1, 1, 1),), ((1, 0, 0), (1, 0, 1)), ((1, 1, 0), (1, 1, 1)))
_ORDER = (3, 1, 4, 2, 6, 0, 5)
_SLOT = (0, 1, 2, 5, 3, 4, 6)
_SHORT = _SLOT[4:]


def _dot(a, b):
    return lax.dot_general(a, b, (((1,), (0,)), ((), ())), preferred_element_type=F32)


def _pack(x):
    return pltpu.bitcast(x.astype(BF), U32)


def _unpack(x):
    return pltpu.bitcast(x, BF)


def _repeat(x, rows, cols):
    return lax.concatenate([lax.concatenate([x] * (rows // 8), 0)] * (cols // 128), 1)


def _true_after(after, rows, cols):
    if after is None:
        return lax.ge(lax.broadcasted_iota(jnp.int32, (rows, cols), 1), 0)
    return lax.ne(_repeat(lax.bitwise_or(lax.bitcast_convert_type(after, jnp.int32), 1), rows, cols), 0)


def _put(ref, r0, c0, val, after=None):
    rows, cols = val.shape
    pltpu.store(ref.at[pl.ds(r0, rows), pl.ds(c0, cols)], val, mask=_true_after(after, rows, cols))


def _tie(val, after):
    if after is None:
        return val
    return lax.select(_true_after(after, *val.shape), val, jnp.zeros_like(val))


def _pad_rows(x, n):
    if x.shape[0] == n:
        return x
    return lax.concatenate([x, jnp.zeros((n - x.shape[0], x.shape[1]), x.dtype)], 0)


def _fold(v):
    return jnp.sum(v.reshape(v.shape[0] // 8, 8, v.shape[1]), axis=0)


def _aligned(i, n):
    return i if isinstance(i, int) else pl.multiple_of(i, n)


def _combine(terms, get):
    out = None
    for sign, bi, bj in terms:
        v = get(bi, bj)
        if v is None:
            continue
        if out is None:
            out = v if sign > 0 else lax.neg(v)
        else:
            out = lax.add(out, v) if sign > 0 else lax.sub(out, v)
    return out


def _operands(table, get, count=7):
    get = functools.cache(get)
    ops = [_combine(table[k], get) for k in _SLOT[:count]]
    return _pack(lax.concatenate([jnp.zeros((16, 128), F32) if v is None else v for v in ops], 1))


def _operands2(table, i, get, count=7):
    return _operands(table, lambda ci, cj: _combine(table[i], lambda bi, bj: get(bi, bj, ci, cj)), count)


def _operand(ref, k, tiles, r0, rows):
    parts = [ref[pl.ds(r0 // 2, rows // 2), pl.ds((t * 7 + _SLOT.index(k)) * 128, 128)] for t in range(tiles)]
    return lax.concatenate(parts, 1)


def _assemble(prod, emit, temps):
    held = {}

    def put(i, v):
        if temps is None:
            held[i] = v
        else:
            _put(temps[i], 0, 0, v)

    def get(i):
        return held[i] if temps is None else temps[i][pl.ds(0, p.shape[0]), pl.ds(0, p.shape[1])]

    p = prod(3)
    put(0, p)
    yield p
    p = prod(1)
    emit(1, 0, lax.add(get(0), p))
    put(1, p)
    yield p
    p = prod(4)
    put(2, p)
    yield p
    p = prod(2)
    emit(0, 1, lax.add(get(2), p))
    put(3, lax.sub(p, get(1)))
    yield p
    p = prod(6)
    put(4, lax.add(lax.sub(get(0), get(2)), p))
    yield p
    p = prod(0)
    emit(0, 0, lax.add(get(4), p))
    put(1, lax.add(get(3), p))
    yield p
    p = prod(5)
    emit(1, 1, lax.add(get(1), p))
    yield p


def _assemble2(leaf, emit, outer_temps, inner_temps):
    leaves = []

    def prod(i):
        c = {}
        leaves.extend(_assemble(functools.partial(leaf, i), lambda ci, cj, v: c.update({(ci, cj): v}), inner_temps))
        return lax.concatenate([lax.concatenate([c[ci, 0], c[ci, 1]], 1) for ci in (0, 1)], 0)

    for _ in _assemble(prod, emit, outer_temps):
        yield from leaves
        leaves.clear()


def _run(matmuls, jobs=(), span=1):
    done = 0
    for i, p in enumerate(matmuls):
        while done < len(jobs) and (done + 0.5) * span / len(jobs) < i + 1:
            r = int(((done + 0.5) * span / len(jobs) - i) * (p.shape[0] // 8)) * 8
            jobs[done](p[r:r + 8, :128])
            done += 1
    assert done == len(jobs)


def _now(jobs):
    for job in jobs:
        job(None)


def _mix(*lists):
    keyed = [((i + 0.5) / len(l), n, job) for n, l in enumerate(lists) for i, job in enumerate(l)]
    return [job for _, _, job in sorted(keyed, key=lambda e: e[:2])]


def _kernel(x_hbm, wqkv_hbm, wo_hbm, w1_hbm, b1_hbm, w2t_hbm, b2_hbm, out_hbm,
            x_s, wqkv_s, wo_s, w1_s, w2t_s, b1_s, b2_s, out_s,
            wot_s, w1t_s, w2p_s, b2c_s, aqkv_s, ao_s, a1_s, a2_s,
            y_s, y2_s, u_s, ur_s, t_s, c_s, h_s, kv_s,
            q_s, k_s, kt_s, v_s, o_s, vmax_s, acc_s, p_s,
            q_st, qw_st, k_st, kt_st, kb_st, v_st, sem):
    D, S = x_hbm.shape
    F = w1_hbm.shape[1]
    DH = D // H
    NQ = S // BQ
    NC = S // 128
    F2 = F // 2 - 512
    tiles = range(0, BQ, 128)
    w_chunks = [(0, 256), (256, 256), (512, 256), (768, 256), (1024, 3 * D - 1024)]

    def accumulate(table, key, v):
        table[key] = table[key] + v if key in table else v

    def project(a_ref, b_ref, r0, rows, emit):
        def prod(k):
            b = _operand(b_ref, k, 2, 0, D - K1 if k in _SHORT else K1)
            return _dot(_unpack(_operand(a_ref, k, 2, r0, rows)), _unpack(_pad_rows(b, K1 // 2)))
        return _assemble(prod, emit, t_s)

    def lhs_jobs(halves, dst, r0):
        def job(r, t, after):
            def get(bi, bj):
                return halves[bi][r:r + 16, bj * K1 + t:bj * K1 + t + 128].astype(F32)
            _put(dst, (r0 + r) // 2, t * 7, _operands(_LHS, get), after)
        return [functools.partial(job, r, t) for t in (0, 128) for r in range(0, halves[0].shape[0], 16)]

    def rhs_jobs(tile, dst):
        def job(r, t, after):
            def get(bi, bj):
                return tile(bi * K1 + r, bj * HB + t) if bi * K1 + r < D else None
            _put(dst, r // 2, t * 7, _operands(_RHS, get, 7 if K1 + r < D else 4), after)
        return [functools.partial(job, r, t) for r in range(0, K1, 16) for t in (0, 128)]

    def norm_jobs(j, cols, total):
        squares = {}

        @functools.cache
        def mean(c):
            return jnp.broadcast_to(jnp.sum(total(c), axis=0, keepdims=True) * (1.0 / D), (8, 128))

        @functools.cache
        def rstd(c):
            return lax.rsqrt(jnp.sum(squares[c], axis=0, keepdims=True) * (1.0 / D) + EPS)

        def centred(r, c, mu):
            return h_s[j][pl.ds(r, 32), pl.ds(c, 128)] - _repeat(mu, 32, 128)

        def square(r, c, after):
            xc = centred(r, c, _tie(mean(c), after))
            accumulate(squares, c, _fold(xc * xc))

        def scale(r, c, after):
            _put(c_s, r, c, centred(r, c, mean(c)) * rstd(c), after)
        return [functools.partial(job, r, c) for job in (square, scale) for r in range(0, D, 32) for c in cols]

    def normed(r, c):
        return c_s[pl.ds(r, 16), pl.ds(c, 128)]

    def in_head(u, shape):
        row = lax.broadcasted_iota(jnp.int32, shape, 0)
        return row >= 4 if u else row < DH

    def query_rows(u, q):
        q = jnp.where(in_head(u, q.shape), q, 0.0)
        if u:
            q = lax.concatenate([jnp.zeros_like(q[:8]), q, jnp.zeros_like(q[:8])], 0)
        return _pack(q)

    def stage_q(i, u, j, t, after):
        q = q_s[pl.ds(_aligned(i * 2 * DH + 24 * u, 8), 32), pl.ds(j * BQ + t, 128)]
        _put(q_st[u][j], 0, t, q, after)
        _put(qw_st[u][j], 8 * u, t, query_rows(u, q), after)

    def stage_k(i, c, r, after):
        _put(k_st[c], r, 0, k_s[pl.ds(_aligned(i * (S // 2) + c * 64 + r, 32), 32), :], after)

    def stage_v(i, u, c, after):
        _put(v_st[u][c], 0, 0, v_s[pl.ds(_aligned(i * 32 + 16 * u, 16), 16), pl.ds(c * 128, 128)], after)

    def spread_keys(src, u, half, d, after, split=False):
        row = jnp.broadcast_to(src[pl.ds(u * DH + d, 1), pl.ds(128 * half, 128)], (8, 128))
        keys = _repeat(_tie(row, after), 128, 128).T
        if split:
            for g in range(8):
                _put(kb_st[u][2 + g], d * 16, 0, keys[g * 16:g * 16 + 16])
        else:
            _put(kb_st[u][half], d * 128, 0, keys)

    def copy_keys(u, c, d, after):
        rows = [kb_st[u][1][pl.ds(e * 128 + c % 8 * 16, 16), :] for e in (d, d + 1)]
        _put(kb_st[u][c - 6], d * 16, 0, lax.concatenate(rows, 0), after)

    def first_norm(j, cols):
        totals = {}

        def widen(r, c, after):
            x = x_s[pl.ds(r, 32), pl.ds(j * BQ + c, 128)].astype(F32)
            _put(h_s[j], r, c, x, after)
            accumulate(totals, c, _fold(x))
        return ([functools.partial(widen, r, c) for c in cols for r in range(0, D, 32)]
                + norm_jobs(j, cols, totals.get))

    def ln1(j):
        return first_norm(j, tiles) + rhs_jobs(normed, y_s[j])

    def features(n, bi):
        c0, width = w_chunks[n]
        cuts = [c0] + [c for c in (D, 2 * D) if c0 < c < c0 + width] + [c0 + width]
        return [(lo + bi * (hi - lo) // 2, (hi - lo) // 2) for lo, hi in zip(cuts, cuts[1:])]

    def wqkv_jobs(n):
        c0, width = w_chunks[n]
        wt = _pad_rows(wqkv_s[:, pl.ds(c0, width)], 2 * K1).T
        halves = [lax.concatenate([wt[r - c0:r - c0 + size] for r, size in features(n, bi)], 0) for bi in (0, 1)]
        return lhs_jobs(halves, aqkv_s, c0 // 2)

    def qkv(*items):
        for j, n in items:
            def emit(bi, bj, v):
                done = 0
                for r, size in features(n, bi):
                    part = v[done:done + size]
                    done += size
                    if r < D:
                        _put(q_s, r, j * BQ + bj * HB, part * (DH ** -0.5 * math.log2(math.e)))
                    else:
                        _put(kv_s[j], r - D, bj * HB, part)
            yield from project(aqkv_s, y_s[j], w_chunks[n][0] // 2, w_chunks[n][1] // 2, emit)

    def swap_halves(k):
        return pltpu.roll(k.reshape(k.shape[0] // 8, 8, 128), 4, 1).reshape(k.shape)

    def finish_k(j):
        def transpose(g, c, after):
            rows = kv_s[j][pl.ds(g * 4 * DH, 128), pl.ds(c, 256)]
            rows = lax.concatenate([_tie(rows[:8], after), rows[8:]], 0)
            _put(k_s, (2 * g * S + j * BQ + c) // 2, 0, swap_halves(_pack(rows.astype(BF).T)))

        def shift(g, c, after):
            k = k_s[pl.ds((2 * g * S + j * BQ + c) // 2, 64), :]
            _put(k_s, ((2 * g + 1) * S + j * BQ + c) // 2, 0, pltpu.roll(_tie(k, after), 128 - 2 * DH, 1))

        def gather(r, after):
            lane = lax.broadcasted_iota(jnp.int32, (32, 128), 1)
            half = j * BQ // 1024 * 128
            k = kt_s[pl.ds(r, 32), pl.ds(half, 128)] if j * BQ % 1024 else None
            for c in tiles:
                tile = kv_s[j][pl.ds(r, 32), pl.ds(c, 128)]
                k = tile if k is None else jnp.where(lane >= (j * BQ + c) // 128 % 8 * 16, tile, k)
            _put(kt_s, r, half, k, after)
        return _mix([functools.partial(gather, r) for r in range(0, D, 32)],
                    [functools.partial(transpose, g, c) for g in range(4) for c in (0, 256)]
                    + [functools.partial(shift, g, c) for g in range(4) for c in tiles])

    def finish_v(j):
        def job(h, after):
            v = jnp.where(in_head(h % 2, (32, BQ)), kv_s[j][pl.ds(D + h * DH // 8 * 8, 32), :], 1.0)
            _put(v_s, h * 16, j * BQ, _pack(v), after)
            top = jnp.max(jnp.abs(v).reshape(4, 8, BQ), axis=0)
            top = functools.reduce(jnp.maximum, [top[:, c:c + 128] for c in tiles])
            _put(vmax_s, 0, 0, jnp.maximum(vmax_s[...], top), after)
        return [functools.partial(job, h) for h in range(H)]

    def load(src, dst, n):
        return pltpu.make_async_copy(src, dst, sem.at[n])

    def wait(copies):
        for cp in copies:
            cp.wait()

    x0_cp = [load(x_hbm.at[:, pl.ds(c, HB)], x_s.at[:, pl.ds(c, HB)], n) for c, n in ((0, 1), (HB, 2))]
    x_cp = [load(x_hbm.at[:, pl.ds(j * BQ, BQ)], x_s.at[:, pl.ds(j * BQ, BQ)], n)
            for j, n in ((1, 5), (2, 6), (3, 6))]
    w_cp = [load(wqkv_hbm.at[:, pl.ds(c, w)], wqkv_s.at[:, pl.ds(c, w)], n)
            for (c, w), n in zip(w_chunks, (0, 3, 4, 4, 5))]
    wo_cp = [load(wo_hbm, wo_s, 6), load(b2_hbm, b2_s, 6)]
    ffn_cp = [load(w1_hbm, w1_s, 0), load(w2t_hbm, w2t_s, 0), load(b1_hbm, b1_s, 0)]
    for cp in w_cp[:1] + x0_cp + w_cp[1:] + x_cp + wo_cp:
        cp.start()
    for ref in (vmax_s, p_s, acc_s[-1], v_st[1][-1]):
        ref[...] = jnp.zeros(ref.shape, ref.dtype)
    for ref in qw_st[1]:
        ref[pl.ds(0, 8), :] = jnp.zeros((8, BQ), U32)

    wait(w_cp[:1])
    _now(wqkv_jobs(0))
    wait(x0_cp[:1])
    _now(first_norm(0, tiles[:2]))
    wait(x0_cp[1:])
    _now(first_norm(0, tiles[2:]) + rhs_jobs(normed, y_s[0]))
    wait(w_cp[1:2])
    _run(qkv((0, 0)))
    _now(wqkv_jobs(1))
    wait(w_cp[2:4])
    _run(qkv((0, 1)))
    _now(wqkv_jobs(2))
    _run(qkv((0, 2)), wqkv_jobs(3), 5)
    wait(w_cp[4:] + x_cp[:1])
    _now(wqkv_jobs(4))
    _run(qkv((0, 3), (0, 4)), ln1(1), 13)
    _run(qkv((1, 1), (1, 2)), _mix(finish_k(0), finish_v(0)), 12)
    wait(x_cp[1:] + wo_cp)
    b2c_s[...] = jnp.broadcast_to(b2_s[...].astype(F32).reshape(1, D), (128, D)).T
    _put(wot_s, 0, 0, _pack(_pad_rows(wo_s[...], 2 * K1).T))
    spread = [functools.partial(spread_keys, kt_s, u, half, d, split=half > 0)
              for half in (0, 1) for u in (0, 1) for d in range(DH)]
    _run(qkv((1, 3), (1, 4)), ln1(2), 13)
    _run(qkv((2, 1), (2, 2), (2, 3)), _mix(ln1(3), finish_k(1)), 19)
    _run(qkv((3, 1), (3, 2), (3, 3)), _mix(finish_k(2), spread[:44], finish_v(1)), 21)
    _run(qkv((1, 0)), finish_k(3), 7)
    wo_jobs = lhs_jobs([_unpack(wot_s[pl.ds(r, D // 4), :]) for r in (0, D // 4)], ao_s, 0)
    _run(qkv((2, 4), (2, 0)), _mix(spread[44:84], wo_jobs), 14)
    _run(qkv((3, 0)), _mix(spread[84:102], finish_v(2)[:10]), 7)
    _run(qkv((3, 4)), _mix(spread[102:], finish_v(2)[10:] + finish_v(3)[:4]), 4)
    _now(finish_v(3)[4:])
    for c in range(NC):
        stage_k(0, c, 0, None)
        stage_k(0, c, 32, None)
    for u in (0, 1):
        for j in range(NQ):
            for t in tiles:
                stage_q(0, u, j, t, None)
        for c in range(NC - u):
            stage_v(0, u, c, None)
    for cp in ffn_cp:
        cp.start()

    def mxu_scores(k, qw, u):
        return _dot(_unpack(k)[:, :32 + 32 * u], _unpack(qw))

    def vpu_scores(u, c, j, hold):
        if c < 8:
            keys = [kb_st[u][0][pl.ds(d * 128 + c * 16, 16), :] for d in range(DH)]
        else:
            keys = [kb_st[u][c - 6][pl.ds(d * 16, 16), :] for d in range(DH)]
        out = []
        for t in tiles:
            acc = None
            for d in range(DH):
                q = q_st[u][j][pl.ds(4 * u + d, 1), pl.ds(t, 128)]
                q = _repeat(hold(t, q), 16, 128) if d == DH - 1 else lax.broadcast_in_dim(q, (16, 128), (0, 1))
                term = lax.mul(keys[d], q)
                acc = term if acc is None else lax.add(acc, term)
            out.append(acc)
        return lax.concatenate(out, 1)

    def values(h, u, c, j, p):
        o = _dot(_unpack(v_st[u][c][...]), p)
        if c:
            o = o + acc_s[j][...]
        if c < NC - 1:
            _put(acc_s[j], 0, 0, o)
        else:
            _put(o_s, _aligned(h * 32 + 32, 32), j * BQ, o)

    def head_pair(i, carry):
        slots = [(u, c, j) for u in (0, 1) for c in range(NC) for j in range(NQ)]
        jobs = {}

        def plan(t, job, *args):
            jobs.setdefault(min(int(t), len(slots) - 1), []).append((t % 1, functools.partial(job, *args)))

        plan(2.5, stage_v, i, 1, NC - 1)
        nxt = jnp.minimum(i + 1, H // 2 - 1)
        _put(kt_st, 0, 0, kt_s[pl.ds(_aligned(nxt * 2 * DH, 8), 2 * DH), :])
        for u in (0, 1):
            t0 = u * NC * NQ
            for d in range(DH):
                plan(t0 + 1 + 29 * (d + 0.5) / DH, spread_keys, kt_st, u, 1, d)
                plan(t0 + 32 + 29 * (d + 0.5) / DH, spread_keys, kt_st, u, 0, d)
            for c in range(NC):
                if u:
                    plan(t0 + NQ * (c + 1) + 0.1, stage_k, nxt, c, 0)
                    plan(t0 + NQ * (c + 1) + 2.6, stage_k, nxt, c, 32)
                if c < NC - u:
                    plan(t0 + NQ * (c + 1) + 1.5, stage_v, nxt, u, c)
                for d in range(0, DH if c >= 8 else 0, 2):
                    span = 1 if (u, c) == (1, NC - 1) else NQ
                    plan(t0 + NQ * (c + 1) - 1 + span * (d + 1) / DH, copy_keys, u, c, d)
            for j in range(NQ):
                for t in tiles:
                    plan(t0 + NQ * (NC - 1) + j + (0 if u else 1 + j) + 0.1 + t / 640, stage_q, nxt, u, j, t)

        always = _true_after(vmax_s[...], 8, 128)
        held = (2 * i - 1, 1, NC - 1, NQ - 1, _unpack(p_s[...]))
        vpu = None
        for n, (u, c, j) in enumerate(slots):
            groups = [g for g in range(7, -1, -1) if g != c % 8 or vpu is None]
            s = mxu_scores(lax.concatenate([k_st[c][pl.ds(g * 8, 8), :] for g in groups], 0), qw_st[u][j][...], u)
            e = jnp.exp2(s)
            p = {g: [e[16 * r + 8:16 * r + 16], e[16 * r:16 * r + 8]] for r, g in enumerate(groups)}
            values(*held)
            held = (2 * i + u, u, c, j, lax.concatenate([x for g in range(8) for x in p.get(g, [vpu])], 0))
            if n + 1 < len(slots):
                vpu = jnp.exp2(vpu_scores(*slots[n + 1], lambda t, q: jnp.where(always, q, s[t // 4:t // 4 + 8, :128])))
            for frac, job in jobs.get(n, []):
                r = int(frac * 14) * 8
                job(s[r:r + 8, :128])
        p_s[...] = _pack(held[-1])
        return carry

    def guarded_tile(n, carry):
        i, cols = n // NC, pl.ds(pl.multiple_of(n % NC * 128, 128), 128)
        for u in (0, 1):
            qw = query_rows(u, q_s[pl.ds(_aligned(i * 2 * DH + 24 * u, 8), 32), cols])
            if u:
                qw = lax.concatenate([jnp.zeros((8, 128), U32), qw], 0)
            s = mxu_scores(swap_halves(k_s[pl.ds(_aligned(i * (S // 2), S // 2), S // 2), :]), qw, u)
            p = jnp.exp2(s - jnp.max(s, axis=0, keepdims=True))
            v = _unpack(v_s[pl.ds(_aligned(i * 32 + 16 * u, 16), 16), pl.ds(0, S)])
            o_s[pl.ds(_aligned(i * 64 + 32 * u + 32, 32), 32), cols] = _dot(v, p)
        return carry

    def heads_jobs(j):
        @functools.cache
        def inverse(h, c):
            den = o_s[pl.ds(h * 32 + 32 + (0 if h % 2 else 31), 1), pl.ds(j * BQ + c, 128)]
            r = pl.reciprocal(den, approx=True)
            return r * (2.0 - den * r)

        def part(h, r, c):
            return o_s[pl.ds(h * 32 + 32 + r - h * DH // 8 * 8, 8), pl.ds(j * BQ + c, 128)] * inverse(h, c)

        def rows8(r, c):
            h0, h1 = r // DH, (r + 7) // DH
            if h0 == h1:
                return part(h0, r, c)
            return jnp.where(in_head(1, (8, 128)), part(h1, r, c), part(h0, r, c))
        return rhs_jobs(lambda r, c: lax.concatenate([rows8(r, c), rows8(r + 8, c)], 0), y_s[2 + j % 2])

    lax.fori_loop(0, H // 2, head_pair, 0)
    values(H - 1, 1, NC - 1, NQ - 1, _unpack(p_s[...]))

    unsafe = _repeat(jnp.where(vmax_s[...] <= SAFE, 0.0, 1.0), 8, BQ)
    for j in range(NQ):
        for h in range(0, H, 2):
            den = jnp.where(in_head(1, (8, BQ)), o_s[pl.ds(h * 32 + 56, 8), pl.ds(j * BQ, BQ)],
                            o_s[pl.ds(h * 32 + 64, 8), pl.ds(j * BQ, BQ)])
            unsafe = jnp.where((den >= 1.0 / SAFE) & (den <= SAFE), unsafe, 1.0)
        if j == NQ - 2:
            for job in heads_jobs(0):
                job(unsafe[:, :128])

    @pl.when(jnp.max(unsafe) > 0.0)
    def _():
        lax.fori_loop(0, H // 2 * NC, guarded_tile, 0)
        _now(heads_jobs(0))

    wait(ffn_cp)

    totals = {}
    written = set()

    def attn_out(j):
        def emit(bi, bj, v):
            v = v + h_s[j][pl.ds(bi * (D // 2), D // 2), pl.ds(bj * HB, HB)]
            _put(h_s[j], bi * (D // 2), bj * HB, v)
            for t in (0, 128):
                accumulate(totals, (j, bj * HB + t), _fold(v[:, t:t + 128]))
        return project(ao_s, y_s[2 + j % 2], 0, D // 2, emit)

    def ln2(j):
        def job(r, i, after):
            def get(bi, bj, ci, cj):
                row = bi * K1 + ci * 128 + r
                if row >= D:
                    return jnp.ones((16, 128), F32) if row == D else None
                return normed(row, bj * HB + cj * 128)
            _put(y2_s[j % 2], (i * 128 + r) // 2, 0, _operands2(_RHS, i, get), after)
        return (norm_jobs(j, tiles, lambda c: totals[j, c]),
                [functools.partial(job, r, i) for i in _ORDER for r in range(0, 128, 16)])

    def transpose_w1(n, c, after):
        cols = pl.ds(256 * n + c, 128)
        b1 = b1_s[...].astype(F32).reshape(1, F)[:, 256 * n + c:256 * n + c + 128]
        bias = jnp.where(lax.broadcasted_iota(jnp.int32, (16, 128), 0) == 0, b1, 0.0).astype(BF)
        first = _unpack(_tie(_pack(w1_s[pl.ds(0, 16), cols]), after))
        w = lax.concatenate([first, w1_s[pl.ds(16, D - 16), cols], bias], 0)
        _put(w1t_s[n % 2], c // 2, 0, _pack(_pad_rows(w, 2 * K1).T))

    def w1_jobs(*chunks):
        def job(n, r, i, after):
            def get(bi, bj, ci, cj):
                rows, cols = pl.ds((bi * 128 + ci * 64 + r) // 2, 8), pl.ds(bj * K1 + cj * 128, 128)
                return _unpack(w1t_s[n % 2][rows, cols]).astype(F32)
            _put(a1_s[n], (i * 64 + r) // 2, 0, _operands2(_LHS, i, get), after)
            written.add(("w1", n, i, r))
        jobs = []
        for n in chunks:
            jobs += [functools.partial(transpose_w1, n + 1, c) for c in (0, 128) if n + 1 < F // 256]
            jobs += [functools.partial(job, n, r, i) for i in _ORDER for r in range(0, 64, 16)]
        return jobs

    def w2_jobs():
        def copy(r, c, after):
            _put(w2p_s, r // 2, c, _pack(w2t_s[pl.ds(r, 32), pl.ds(c, 256)]), after)

        def job(r, c, i, after):
            def get(bi, bj, ci, cj):
                if cj and c >= F2:
                    return None
                rows = pl.ds((bi * (D // 2) + ci * (D // 4) + r) // 2, 8)
                return _unpack(w2p_s[rows, pl.ds(bj * (F // 2) + cj * 512 + c, 128)]).astype(F32)
            _put(a2_s, (i * (D // 4) + r) // 2, c * 7, _operands2(_LHS, i, get, 7 if c < F2 else 4), after)
            written.add(("w2", i, r, c))
        return ([functools.partial(copy, r, c) for r in range(0, D, 32) for c in range(0, F, 256)],
                [functools.partial(job, r, c, i)
                 for i in _ORDER for r in range(0, D // 4, 16) for c in range(0, 512, 128)])

    def up(j, chunks=range(F // 256)):
        for n in chunks:
            def leaf(i, k):
                assert ("w1", n, i, 48) in written
                return _dot(_unpack(_operand(a1_s[n], k, 1, i * 64, 64)),
                            _unpack(_operand(y2_s[j % 2], k, 1, i * 128, 128)))

            def emit(bi, bj, v):
                v = jnp.maximum(v, 0.0)
                _put(u_s[j % 2], 256 * n + 128 * bi, bj * HB, v * v)
            yield from _assemble2(leaf, emit, t_s[:5], None)

    def hidden_jobs(j):
        def job(r, i, after):
            def get(bi, bj, ci, cj):
                if ci and r >= F2:
                    return None
                return u_s[j % 2][pl.ds(bi * (F // 2) + ci * 512 + r, 16), pl.ds(bj * HB + cj * 128, 128)]
            _put(ur_s[j % 2], (i * 512 + r) // 2, 0, _operands2(_RHS, i, get, 7 if r < F2 else 4), after)
            written.add(("u", j, i, r))
        return [functools.partial(job, r, i) for i in _ORDER for r in range(0, 512, 16)]

    out_cp = []

    def store(rows, cols):
        out_cp.append(pltpu.make_async_copy(out_s.at[rows, cols], out_hbm.at[rows, cols], sem.at[1]))
        out_cp[-1].start()

    def down(j):
        def leaf(i, k):
            assert ("u", j, i, 496) in written and ("w2", i, D // 4 - 16, 384) in written
            width = F2 if k in _SHORT else 512
            return _dot(_unpack(_operand(a2_s, k, width // 128, i * (D // 4), D // 4)),
                        _unpack(_operand(ur_s[j % 2], k, 1, i * 512, width)))

        def emit(bi, bj, v):
            rows, cols = pl.ds(bi * (D // 2), D // 2), pl.ds(j * BQ + bj * HB, HB)
            v = v + h_s[j][rows, pl.ds(bj * HB, HB)] + jnp.tile(b2c_s[rows, :], (1, HB // 128))
            if (j, bi, bj) == (NQ - 1, 1, 1):
                for ci, cj in ((1, 0), (0, 1), (0, 0), (1, 1)):
                    rows, cols = pl.ds(D // 2 + ci * (D // 4), D // 4), pl.ds(j * BQ + HB + cj * 128, 128)
                    out_s[rows, cols] = v[ci * (D // 4):(ci + 1) * (D // 4), cj * 128:cj * 128 + 128].astype(BF)
                    store(rows, cols)
                return
            out_s[rows, cols] = v.astype(BF)
            if j == NQ - 1:
                store(rows, cols)
        yield from _assemble2(leaf, emit, t_s[:5], t_s[5:])
        if j < NQ - 1:
            store(pl.ds(0, D), pl.ds(j * BQ, BQ))

    transpose_w1(0, 0, None)
    transpose_w1(0, 128, None)
    norm, rhs = ln2(0)
    _run(attn_out(0), _mix(heads_jobs(1), w1_jobs(0)), 6)
    _run(attn_out(1), _mix(heads_jobs(2), norm), 6)
    _run(attn_out(2), _mix(rhs, w1_jobs(1)), 6)
    norm, rhs = ln2(1)
    _run(up(0, range(6)), _mix(w1_jobs(2, 3, 4, 5, 6), norm[:84]), 280)
    _run(up(0, range(6, 7)), _mix(norm[84:], heads_jobs(3)), 45)
    _run(attn_out(3), rhs, 6)
    hidden = [hidden_jobs(j) for j in range(NQ)]
    w2_copy, w2 = w2_jobs()
    _run(up(1), _mix(w2_copy + w2[:3 * 28], hidden[0][:3 * 32]), 342)
    _run(down(0), _mix(w2[3 * 28:], hidden[0][3 * 32:]) + hidden[1][:2 * 32], 47)
    norm, rhs = ln2(2)
    _run(down(1), _mix(hidden[1][2 * 32:], norm) + rhs, 46)
    norm, rhs = ln2(3)
    _run(up(2), norm + rhs, 330)
    _run(up(3), hidden[2][:4 * 32], 335)
    _run(down(2), hidden[2][4 * 32:] + hidden[3][:4 * 32], 46)
    _run(down(3), hidden[3][4 * 32:], 28)
    wait(out_cp)


@jax.jit
def pallas_sequential_preLN__softmax_full_mha__dense_activation_squared_relu__prompt_kernel(
    A_x: jax.Array,
    A_wqkv: jax.Array,
    A_wo: jax.Array,
    B_x: jax.Array,
    B_w1: jax.Array,
    B_b1: jax.Array,
    B_w2: jax.Array,
    B_b2: jax.Array,
):
    del B_x
    _, S, D = A_x.shape
    F = B_w1.shape[1]
    NQ, NC, DH = S // BQ, S // 128, D // H
    vmem = pltpu.VMEM
    hbm = pl.BlockSpec(memory_space=pltpu.HBM)
    scratch = [
        vmem((D, S + 256), BF),
        vmem((D, 3 * D), BF),
        vmem((D, D), BF),
        vmem((D, F), BF),
        vmem((D, F), BF),
        vmem((F,), BF),
        vmem((D,), BF),
        vmem((D, S + 256), BF),
        vmem((D // 2, 2 * K1), U32),
        [vmem((128, 2 * K1), U32)] * 2,
        vmem((D // 2, F), U32),
        vmem((D, 128), F32),
        vmem((3 * D // 4, 7 * K1), U32),
        vmem((D // 4, 7 * K1), U32),
        [vmem((7 * 32, 7 * 128), U32)] * (F // 256),
        vmem((7 * D // 8, 7 * 512), U32),
        [vmem((K1 // 2, 7 * HB), U32)] * NQ,
        [vmem((7 * 64, 7 * 128), U32)] * 2,
        [vmem((F, BQ), F32)] * 2,
        [vmem((7 * 256, 7 * 128), U32)] * 2,
        [vmem((D // 2, HB), F32)] * 10,
        vmem((D, BQ), F32),
        [vmem((D, BQ), F32)] * NQ,
        [vmem((2 * D, BQ), F32)] * NQ,
        vmem((D, S + 128), F32),
        vmem((H // 2 * S // 2, 128), U32),
        vmem((D, 256), F32),
        vmem((H * 16, S + 128), U32),
        vmem((H * 32 + 32, S + 128), F32),
        vmem((8, 128), F32),
        [vmem((32, BQ), F32)] * NQ,
        vmem((64, BQ), U32),
        [[vmem((32, BQ), F32)] * NQ] * 2,
        [[vmem((16 + 16 * u, BQ), U32)] * NQ for u in (0, 1)],
        [vmem((64, 128), U32)] * NC,
        vmem((2 * DH, 256), F32),
        [[vmem((DH * n, 128), F32) for n in [128, 128] + [16] * 8]] * 2,
        [[vmem((16, 128), U32)] * NC] * 2,
        pltpu.SemaphoreType.DMA((7,)),
    ]
    out_t = pl.pallas_call(
        _kernel,
        out_shape=jax.ShapeDtypeStruct((D, S), A_x.dtype),
        in_specs=[hbm] * 7,
        out_specs=hbm,
        scratch_shapes=scratch,
        compiler_params=pltpu.CompilerParams(vmem_limit_bytes=120 << 20),
    )(A_x[0].T, A_wqkv, A_wo, B_w1, B_b1, B_w2.T, B_b2)
    return out_t.T[None]
```
